```python
import os as _os
_os.environ.setdefault("JAX_PLATFORMS", "cpu")
import jax
import jax.numpy as jnp

def _softmax(x, axis=-1):
    return jax.nn.softmax(x, axis=axis)
def _gelu(x):
    return jax.nn.gelu(x, approximate=True)
def _silu(x):
    return jax.nn.silu(x)
def _sigmoid(x):
    return jax.nn.sigmoid(x)
def _layernorm(x, axis=-1, eps=1e-5):
    m = jnp.mean(x, axis=axis, keepdims=True)
    v = jnp.var(x, axis=axis, keepdims=True)
    return (x - m) / jnp.sqrt(v + eps)
def _scatter_add(tgt, idx, src, axis=0):
    return tgt.at[idx].add(src)
def _segment_sum(src, seg, n):
    return jax.ops.segment_sum(src, seg, n)
class _Rng:
    def __init__(self, key):
        self._k = key
    def _next(self):
        self._k, sub = jax.random.split(self._k)
        return sub
    def normal(self, shape):
        return jax.random.normal(self._next(), shape, dtype=jnp.bfloat16)
    def randint(self, lo, hi, shape):
        return jax.random.randint(self._next(), shape, lo, hi, dtype=jnp.int32)
    def uniform(self, shape, lo=0.0, hi=1.0):
        return jax.random.uniform(self._next(), shape, jnp.bfloat16, lo, hi)
    def permutation(self, n):
        return jax.random.permutation(self._next(), n)


kernel_name = 'parallel_sum__grouped_kv_mqa__dense_activation_silu__prompt'

def setup_inputs():
    _rng = _Rng(jax.random.key(int.from_bytes(__import__("os").urandom(4), "little")))
    _w = (lambda a: (lambda t: t.astype(jnp.bfloat16) if jnp.issubdtype(t.dtype, jnp.floating) else t)(jnp.asarray(a)))
    def _A_setup():
        B, S, D, H = 1, 2048, 512, 32
        Dh = D // H
        return {
            "x": _w((lambda *s: _rng.normal(s) * 0.05)(B, S, D)),
            "wq": _w((lambda *s: _rng.normal(s) * 0.05)(D, H * Dh)),
            "wk": _w((lambda *s: _rng.normal(s) * 0.05)(D, Dh)),
            "wv": _w((lambda *s: _rng.normal(s) * 0.05)(D, Dh)),
            "wo": _w((lambda *s: _rng.normal(s) * 0.05)(H * Dh, D)),
        }
    _A_in = _A_setup()

    def _B_setup():
        B, S, D, F = 1, 2048, 512, 1376
        return {
            "x": _w((lambda *s: _rng.normal(s) * 0.05)(B, S, D)),
            "w1": _w((lambda *s: _rng.normal(s) * 0.05)(D, F) * (D ** -0.5)),
            "w2": _w((lambda *s: _rng.normal(s) * 0.05)(F, D) * (F ** -0.5)),
        }
    _B_in = _B_setup()

    return {
        "A_x": _A_in["x"],
        "A_wq": _A_in["wq"],
        "A_wk": _A_in["wk"],
        "A_wv": _A_in["wv"],
        "A_wo": _A_in["wo"],
        "B_x": _B_in["x"],
        "B_w1": _B_in["w1"],
        "B_w2": _B_in["w2"],
    }

def reference(A_x, A_wq, A_wk, A_wv, A_wo, B_x, B_w1, B_w2):
    def _A_ref(x, wq, wk, wv, wo):
        B, S, D = x.shape
        H = 32
        Dh = D // H
        q = (lambda x, *d: x.transpose(*d))((x @ wq).reshape(B, S, H, Dh), 0, 2, 1, 3)
        k = x @ wk
        v = x @ wv
        scores = jnp.einsum("bhqd,bkd->bhqk", q, k) * (Dh ** -0.5)
        p = _softmax(scores, axis=-1)
        o = jnp.einsum("bhqk,bkd->bhqd", p, v)
        return (lambda x, *d: x.transpose(*d))(o, 0, 2, 1, 3).reshape(B, S, H * Dh) @ wo

    def _B_ref(x, w1, w2):
        h = jnp.einsum("bsd,df->bsf", x, w1)
        h = _silu(h)
        out = jnp.einsum("bsf,fd->bsd", h, w2)
        return out

    x = A_x
    xn = _layernorm(x, axis=-1)
    return x + _A_ref(xn, A_wq, A_wk, A_wv, A_wo) + _B_ref(xn, B_w1, B_w2)
```

```python
import functools, math
import jax, jax.numpy as jnp
from jax import lax
from jax.experimental import pallas as pl
from jax.experimental.pallas import tpu as pltpu

S, D, H, DH, F = 2048, 512, 32, 16, 1376
FP = 1408
NF = FP // 128
LOG2E = math.log2(math.e)
CSC = DH ** -0.5 * LOG2E
FS = 3960.0
BMAX = 64.0
MAGIC = 12582912.0
f32, bf16, i32, i8, u32 = jnp.float32, jnp.bfloat16, jnp.int32, jnp.int8, jnp.uint32
NT = (((1,), (1,)), ((), ()))
TN = (((0,), (0,)), ((), ()))

def _ln(x):
    x = x.astype(f32)
    m = jnp.mean(x, axis=-1, keepdims=True)
    xc = x - m
    v = jnp.mean(xc * xc, axis=-1, keepdims=True)
    return xc * lax.rsqrt(v + 1e-5)

def _limbs(y):
    bits = pltpu.bitcast(y + MAGIC, i32)
    hi = (bits + 128) >> 8
    hi8 = hi << 3
    lo2 = (((bits << 24) >> 24) + 8) >> 4
    return hi8, hi, bits, lo2

def _silu(h):
    e = jnp.exp2(h * (-LOG2E))
    return h * pl.reciprocal(1.0 + e, approx=True)

def _pk(x):
    return pltpu.bitcast(x, u32)
def _upk(x):
    return pltpu.bitcast(x, bf16)

def build(TQ=512, KC=256, force_slow=False, HB=1, nloop=None, foff=0,
          XB=(0, 256, 1024, 2048), LN0=256, RLN=64, KVL=2, QL1=2, QL2=8, OB=256, pvfirst=False,
          wstart=None):
    NG = S // TQ
    NC = S // KC
    RB = S // (H // HB)
    NXB = len(XB) - 1
    NO = S // OB
    nloop_ = nloop if nloop is not None else H // HB
    wstart = NXB if wstart is None else wstart
    def kernel(x_hbm, wq_hbm, wkT_hbm, wvT_hbm, wo_hbm, w1T_hbm, w2_hbm, o_hbm,
               x_scr, wq_scr, wkvT_scr, wo_scr, w1T_scr, w2_scr, sems, osems,
               xn_scr, wqT_scr, kT_scr, k8_scr, kb_scr, vT_scr,
               q8_scr, sq_scr, oT_scr, acc_scr, hid_scr, p_scr, l_scr, out_scr):
        P = [p_scr.at[k] for k in range(2)]
        L = [l_scr.at[k] for k in range(2)]

        def x_copy(c):
            lo, hi = XB[c], XB[c + 1]
            return pltpu.make_async_copy(x_hbm.at[pl.ds(lo, hi - lo), :], x_scr.at[pl.ds(lo, hi - lo), :], sems.at[c])
        wk_copy = pltpu.make_async_copy(wkT_hbm, wkvT_scr.at[pl.ds(0, DH), :], sems.at[NXB])
        wv_copy = pltpu.make_async_copy(wvT_hbm, wkvT_scr.at[pl.ds(DH, DH), :], sems.at[NXB + 1])
        wq_copy = pltpu.make_async_copy(wq_hbm, wq_scr, sems.at[NXB + 2])
        w1_copy = pltpu.make_async_copy(w1T_hbm, w1T_scr.at[pl.ds(0, F), :], sems.at[NXB + 3])
        w2_copy = pltpu.make_async_copy(w2_hbm, w2_scr.at[pl.ds(0, F), :], sems.at[NXB + 4])
        wo_copy = pltpu.make_async_copy(wo_hbm, wo_scr, sems.at[NXB + 5])
        def o_copy(k):
            return pltpu.make_async_copy(out_scr.at[pl.ds(k * OB, OB), :], o_hbm.at[pl.ds(k * OB, OB), :], osems.at[k])

        x_copy(0).start()
        wq_copy.start()
        wk_copy.start(); wv_copy.start()
        for c in range(1, NXB):
            x_copy(c).start()
        w1T_scr[pl.ds(F, FP - F), :] = jnp.zeros((FP - F, D), bf16)
        w2_scr[pl.ds(F, FP - F), :] = jnp.zeros((FP - F, D), bf16)

        QG = 4
        HG = H // QG
        NT_ = S // 128
        NM = NT_ * QG
        def ln_piece(r0, n):
            xn = _ln(x_scr[r0:r0 + n, :]).astype(bf16)
            xn_scr[r0 // 2:(r0 + n) // 2, :] = _pk(xn)
        def q_mm(m):
            t, gq = divmod(m, QG)
            xn = _upk(xn_scr[t * 64:(t + 1) * 64, :])
            w = _upk(wqT_scr[gq * 64:(gq + 1) * 64, :])
            qT = lax.dot_general(w, xn, NT, preferred_element_type=f32)
            acc_scr[(t % 3) * D + gq * 128:(t % 3) * D + (gq + 1) * 128, 0:128] = qT
            p_scr[t % 2, gq * 64:(gq + 1) * 64, 0:128] = _pk((qT * qT).astype(bf16))
        def kv_mm(t, st):
            xn = _upk(xn_scr[t * 64:(t + 1) * 64, :])
            r = lax.dot_general(wkvT_scr[...], xn, NT, preferred_element_type=f32)
            kT = r[0:DH, :]
            kT_scr[:, t * 128:(t + 1) * 128] = kT
            vT_scr[:, t * 128:(t + 1) * 128] = _pk(r[DH:2 * DH, :].astype(bf16))
            am = jnp.abs(r)
            st["amax"] = am if st["amax"] is None else jnp.maximum(st["amax"], am)
            k2 = jnp.sum(kT * kT, axis=0, keepdims=True)
            st["kn2"] = k2 if st["kn2"] is None else jnp.maximum(st["kn2"], k2)
        def k_stats(st):
            amax = st["amax"]
            kmax = jnp.max(jnp.max(amax[0:DH, :], axis=0, keepdims=True), axis=1, keepdims=True)
            st["vmax"] = jnp.max(jnp.max(amax[DH:2 * DH, :], axis=0, keepdims=True), axis=1, keepdims=True)
            st["kn2"] = jnp.max(st["kn2"], axis=1, keepdims=True)
            kmax = jnp.maximum(kmax, 1e-30)
            st["kscale"] = FS / kmax
            kfac = kmax * (256.0 * CSC / FS)
            sq_scr[H:H + 8, 0:TQ] = jnp.broadcast_to(kfac, (8, TQ))
        def k_quant(c, st):
            hi8, hi, lo, lo2 = _limbs(kT_scr[:, c * 128:(c + 1) * 128] * st["kscale"])
            k8T = jnp.concatenate([hi8, hi8, hi8, hi8, lo, hi, lo2, jnp.zeros_like(hi)], axis=0)
            k8_scr[c * 128:(c + 1) * 128, :] = k8T.T.astype(i8)
        def q_norm(t, st):
            gsel = jnp.where((lax.broadcasted_iota(i32, (H, D), 1) >> 4)
                             == lax.broadcasted_iota(i32, (H, D), 0), 1.0, 0.0).astype(bf16)
            n2 = jnp.dot(gsel, _upk(p_scr[t % 2, 0:D // 2, 0:128]), preferred_element_type=f32)
            n2 = n2 * (1.0 + 2.0 ** -6) + 1e-36
            st["qn2"] = n2 if st["qn2"] is None else jnp.maximum(st["qn2"], n2)
            inv = lax.rsqrt(n2) * FS
            sq_scr[H + 8:2 * H + 8, t * 128:(t + 1) * 128] = inv
            sq_scr[0:H, t * 128:(t + 1) * 128] = 1.0 / inv
        def q_quant(m):
            t, gq = divmod(m, QG)
            for hh in range(gq * HG, (gq + 1) * HG):
                q = acc_scr[(t % 3) * D + hh * DH:(t % 3) * D + (hh + 1) * DH, 0:128]
                hi8, hi, lo, lo2 = _limbs(q * sq_scr[H + 8 + hh:H + 9 + hh, t * 128:(t + 1) * 128])
                q8 = jnp.concatenate([hi8, hi8, hi8, hi8, hi, lo, lo2, jnp.zeros_like(hi)], axis=0)
                q8_scr[hh, :, t * 128:(t + 1) * 128] = q8.astype(i8)

        st = dict(amax=None, kn2=None, qn2=None)
        x_copy(0).wait()
        for r0 in range(0, LN0, 32):
            ln_piece(r0, 32)
        ln_done = LN0
        wq_copy.wait(); wk_copy.wait(); wv_copy.wait()
        waited = 1
        kv_done = 0
        kv_ready_at = {t: -10 for t in range(LN0 // 128)}
        stats_at = None
        kq_done = 0
        for m in range(NM + QL2):
            r1 = min(S, ln_done + RLN)
            while ln_done < S and r1 > XB[waited]:
                x_copy(waited).wait()
                waited += 1
                if waited == wstart:
                    w1_copy.start(); w2_copy.start(); wo_copy.start()
            if m < QG:
                if m == 0:
                    wqT_scr[0:64, :] = _pk(wq_scr[:, 0:128].T)
                if m + 1 < QG:
                    wqT_scr[(m + 1) * 64:(m + 2) * 64, :] = _pk(wq_scr[:, (m + 1) * 128:(m + 2) * 128].T)
            if m < NM:
                assert (m // QG + 1) * 128 <= ln_done
                q_mm(m)
            if kv_done < NT_ and kv_done in kv_ready_at and m >= kv_ready_at[kv_done] + KVL:
                kv_mm(kv_done, st)
                kv_done += 1
                if kv_done == NT_:
                    stats_at = m + 2
            if (m - QL1) % QG == 0 and 0 <= (m - QL1) // QG - 1 < NT_:
                q_norm((m - QL1) // QG - 1, st)
            if 0 <= m - QL2 < NM:
                q_quant(m - QL2)
            if stats_at is not None and m == stats_at:
                k_stats(st)
            if stats_at is not None and m >= stats_at + 2 and kq_done < NT_:
                k_quant(kq_done, st)
                kq_done += 1
            for r0 in range(ln_done, r1, 32):
                ln_piece(r0, 32)
            for t in range(ln_done // 128, r1 // 128):
                kv_ready_at[t] = m
            ln_done = r1
        assert kq_done == NT_, kq_done
        kn2, qn2m, vmax = st["kn2"], st["qn2"], st["vmax"]
        qn2m = jnp.max(jnp.max(qn2m, axis=0, keepdims=True), axis=1, keepdims=True)
        bound2 = qn2m * kn2 * (CSC * CSC)
        okv = jnp.where((bound2 <= BMAX * BMAX) & (vmax <= 2.0 ** 40) & (vmax >= 2.0 ** -30), 1, 0).astype(i32)
        ok = okv[0, 0] > (1 if force_slow else 0)
        w1_copy.wait(); w2_copy.wait(); wo_copy.wait()

        def qk(h, g, c, slot, lacc, sq):
            q = q8_scr[h, :, g * TQ:(g + 1) * TQ]
            s = jnp.dot(k8_scr[c * KC:(c + 1) * KC, :], q, preferred_element_type=i32).astype(f32)
            p = jnp.exp2(s * sq)
            ls = jnp.sum(p.reshape(KC // 8, 8, TQ), axis=0)
            lacc = ls if lacc is None else lacc + ls
            P[slot][c * KC // 2:(c + 1) * KC // 2, :] = _pk(p.astype(bf16))
            return lacc
        def pv(c, slot, acc):
            p = _upk(P[slot][c * KC // 2:(c + 1) * KC // 2, :])
            v = _upk(vT_scr[:, c * KC:(c + 1) * KC])
            o = jnp.dot(v, p, preferred_element_type=f32)
            return o if acc is None else o + acc

        def ffn_piece(rb, t):
            j = t // 2
            r0 = rb * RB if isinstance(rb, int) else pl.multiple_of(rb * RB, RB)
            rh = rb * (RB // 2) if isinstance(rb, int) else pl.multiple_of(rb * (RB // 2), RB // 2)
            if t % 2 == 0:
                xk = _upk(xn_scr[pl.ds(rh, RB // 2), :])
                hh = lax.dot_general(xk, w1T_scr[j * 128:(j + 1) * 128, :], NT, preferred_element_type=f32)
                hid_scr[:, j * 128:(j + 1) * 128] = _pk(_silu(hh).astype(bf16))
            else:
                hb = _upk(hid_scr[:, j * 128:(j + 1) * 128])
                part = jnp.dot(hb, w2_scr[j * 128:(j + 1) * 128, :], preferred_element_type=f32)
                if j == 0:
                    acc_scr[pl.ds(r0, RB), :] = part + x_scr[pl.ds(r0, RB), :].astype(f32)
                else:
                    acc_scr[pl.ds(r0, RB), :] = acc_scr[pl.ds(r0, RB), :] + part

        def ffn_order():
            order = [0, 2]
            for j in range(NF):
                order.append(2 * j + 1)
                if j + 2 < NF:
                    order.append(2 * (j + 2))
            return order

        def stage(hq, gq, sq_slot, hp, gp, sp_slot, filler):
            acc = None
            lacc = None
            if hq is not None:
                sq = sq_scr[pl.ds(hq, 1), gq * TQ:(gq + 1) * TQ] * sq_scr[H:H + 1, 0:TQ]
            for c in range(NC):
                if pvfirst and hp is not None:
                    acc = pv(c, sp_slot, acc)
                if hq is not None:
                    lacc = qk(hq, gq, c, sq_slot, lacc, sq)
                for fn_ in filler.get(c, []):
                    fn_()
                if not pvfirst and hp is not None:
                    acc = pv(c, sp_slot, acc)
            if hq is not None:
                L[sq_slot][...] = lacc
            if hp is not None:
                l = jnp.sum(L[sp_slot][...], axis=0, keepdims=True)
                rr = (hp + 1) * 8 if isinstance(hp, int) else pl.multiple_of((hp + 1) * 8, 8)
                oT_scr[pl.ds(rr, 8), gp * TQ:(gp + 1) * TQ] = _pk((acc / l).astype(bf16))

        def oproj(k):
            oT = _upk(oT_scr[8:8 + D // 2, k * OB:(k + 1) * OB])
            attn = lax.dot_general(oT, wo_scr[...], TN, preferred_element_type=f32)
            out_scr[k * OB:(k + 1) * OB, :] = (attn + acc_scr[k * OB:(k + 1) * OB, :]).astype(bf16)
            o_copy(k).start()
        NO1 = (S - TQ) // OB

        @pl.when(ok)
        def _fast():
            def body(it, carry):
                nst = HB * NG
                tot = nst * NC
                fl = [dict() for _ in range(nst)]
                order = ffn_order()
                for k, t in enumerate(order):
                    pos = (k * tot) // len(order) + foff
                    fl[pos // NC].setdefault(pos % NC, []).append(functools.partial(ffn_piece, it, t))
                for u in range(nst):
                    h = it * HB + u // NG
                    g = u % NG
                    hp, gp = (h - 1, NG - 1) if g == 0 else (h, g - 1)
                    stage(h, g, u % 2, hp, gp, (u + 1) % 2, fl[u])
                return carry
            lax.fori_loop(0, nloop_, body, 0)
            fl = {}
            for k in range(min(NO1, NC // 2)):
                fl.setdefault(2 * k, []).append(functools.partial(oproj, k))
            stage(None, None, None, H - 1, NG - 1, 1, fl)
            for k in range(min(NO1, NC // 2), NO):
                oproj(k)

        @pl.when(jnp.logical_not(ok))
        def _slow():
            for g in range(NG):
                xn = _upk(xn_scr[g * TQ // 2:(g + 1) * TQ // 2, :])
                kb_scr[g * TQ:(g + 1) * TQ, :] = lax.dot_general(
                    xn, wkvT_scr[0:DH, :], NT, preferred_element_type=f32).astype(bf16)
            for g in range(NG):
                def head(h, carry):
                    w = _upk(wqT_scr[pl.ds(pl.multiple_of(h * (DH // 2), DH // 2), DH // 2), :])
                    xn = _upk(xn_scr[g * TQ // 2:(g + 1) * TQ // 2, :])
                    q = (lax.dot_general(w, xn, NT, preferred_element_type=f32) * CSC).astype(bf16)
                    sT = jnp.dot(kb_scr[...], q, preferred_element_type=f32)
                    m = jnp.max(sT, axis=0, keepdims=True)
                    p = jnp.exp2(sT - m)
                    l = jnp.sum(p, axis=0, keepdims=True)
                    oT = jnp.dot(_upk(vT_scr[...]), p.astype(bf16), preferred_element_type=f32)
                    rr = pl.multiple_of((h + 1) * 8, 8)
                    oT_scr[pl.ds(rr, 8), g * TQ:(g + 1) * TQ] = _pk((oT / l).astype(bf16))
                    return carry
                lax.fori_loop(0, H, head, 0)
            def fbody(rb, carry):
                for t in range(2 * NF):
                    ffn_piece(rb, t)
                return carry
            lax.fori_loop(0, S // RB, fbody, 0)
            for k in range(NO):
                oproj(k)

        for k in range(NO):
            o_copy(k).wait()

    @jax.jit
    def fn(A_x, A_wq, A_wk, A_wv, A_wo, B_x, B_w1, B_w2):
        x = A_x.reshape(S, D)
        anyspec = pl.BlockSpec(memory_space=pl.ANY)
        out = pl.pallas_call(
            kernel,
            in_specs=[anyspec] * 7,
            out_specs=anyspec,
            out_shape=jax.ShapeDtypeStruct((S, D), bf16),
            scratch_shapes=[
                pltpu.VMEM((S, D), bf16),
                pltpu.VMEM((D, D), bf16),
                pltpu.VMEM((2 * DH, D), bf16),
                pltpu.VMEM((D, D), bf16),
                pltpu.VMEM((FP, D), bf16),
                pltpu.VMEM((FP, D), bf16),
                pltpu.SemaphoreType.DMA((NXB + 6,)),
                pltpu.SemaphoreType.DMA((NO,)),
                pltpu.VMEM((S // 2, D), u32),
                pltpu.VMEM((D // 2, D), u32),
                pltpu.VMEM((DH, S), f32),
                pltpu.VMEM((S, 128), i8),
                pltpu.VMEM((S, DH), bf16),
                pltpu.VMEM((8, S), u32),
                pltpu.VMEM((H, 128, S), i8),
                pltpu.VMEM((2 * H + 8, S), f32),
                pltpu.VMEM(((H + 1) * 8, S), u32),
                pltpu.VMEM((S, D), f32),
                pltpu.VMEM((RB // 2, FP), u32),
                pltpu.VMEM((2, S // 2, TQ), u32),
                pltpu.VMEM((2, 8, TQ), f32),
                pltpu.VMEM((S, D), bf16),
            ],
            compiler_params=pltpu.CompilerParams(vmem_limit_bytes=100 * 1024 * 1024),
        )(x, A_wq, A_wk.T, A_wv.T, A_wo, B_w1.T, B_w2)
        return out.reshape(1, S, D)
    return fn


pallas_parallel_sum__grouped_kv_mqa__dense_activation_silu__prompt_kernel = build(HB=2)
```

```python
import functools
import math

import jax
import jax.numpy as jnp
from jax import lax
from jax.experimental import pallas as pl
from jax.experimental.pallas import tpu as pltpu

S, D, H, DH, F = 2048, 512, 32, 16, 1376
LOG2E = math.log2(math.e)
CSC = DH ** -0.5 * LOG2E
FS = 3960.0
BMAX = 64.0
MAGIC = 12582912.0
f32, bf16, i32, i8, u32 = jnp.float32, jnp.bfloat16, jnp.int32, jnp.int8, jnp.uint32
NT = (((1,), (1,)), ((), ()))
TN = (((0,), (0,)), ((), ()))

TQ, KC = 512, 256
NG, NC = S // TQ, S // KC
HB = 4
RB = S // (H // HB)
RS = 64
JL = 8
FL = JL * 128
FR, FRP = F - FL, 384
XB = (0, 256, 512, 1024, 2048)
NXB = len(XB) - 1
OB = 256
NO = S // OB
QG = 4
HG = H // QG
NTL = S // 128
NM = NTL * QG
NU = NTL * (FRP // 128)


def _ln(x):
    x = x.astype(f32)
    m = jnp.mean(x, axis=-1, keepdims=True)
    xc = x - m
    v = jnp.mean(xc * xc, axis=-1, keepdims=True)
    return xc * lax.rsqrt(v + 1e-5)


def _limbs(y):
    bits = pltpu.bitcast(y + MAGIC, i32)
    hi = (bits + 128) >> 8
    lo2 = (((bits << 24) >> 24) + 8) >> 4
    return hi << 3, hi, bits, lo2


def _silu(h):
    d = 1.0 + jnp.exp2(jnp.minimum(h * (-LOG2E), 126.0))
    r = pl.reciprocal(d, approx=True)
    r = r * (2.0 - d * r)
    return h * r


def _pk(x):
    return pltpu.bitcast(x, u32)


def _upk(x):
    return pltpu.bitcast(x, bf16)


def _off(k, n):
    return k * n if isinstance(k, int) else pl.multiple_of(k * n, n)


def _prologue_slots():
    slots, nq, nu = [], 0, 0
    while nq < NM or nu < NU:
        if nq < NM and (len(slots) < 12 or nu >= NU - 6 or nu * 4 >= (nq - 12) * 3):
            slots.append(("q", nq))
            nq += 1
        else:
            slots.append(("u", nu))
            nu += 1
    return slots


def _ffn_order():
    order = [0, 2]
    for j in range(JL):
        order.append(2 * j + 1)
        if j + 2 < JL:
            order.append(2 * (j + 2))
    return order


def _kernel(x_hbm, wq_hbm, wkT_hbm, wvT_hbm, wo_hbm, w1T_hbm, w2_hbm, o_hbm,
            x_scr, wq_scr, wkvT_scr, wo_scr, w1T_scr, w2_scr, w1r_scr, w2r_scr, sems, osems,
            xn_scr, wqT_scr, kT_scr, k8_scr, kb_scr, vT_scr,
            q8_scr, sq_scr, oT_scr, acc_scr, hid_scr, hr_scr, p_scr, l_scr, out_scr,
            w1p_scr, w2p_scr):
    P = [p_scr.at[k] for k in range(2)]
    L = [l_scr.at[k] for k in range(2)]

    def x_copy(c):
        lo, n = XB[c], XB[c + 1] - XB[c]
        return pltpu.make_async_copy(x_hbm.at[pl.ds(lo, n), :], x_scr.at[pl.ds(lo, n), :], sems.at[c])

    wk_copy = pltpu.make_async_copy(wkT_hbm, wkvT_scr.at[pl.ds(0, DH), :], sems.at[NXB])
    wv_copy = pltpu.make_async_copy(wvT_hbm, wkvT_scr.at[pl.ds(DH, DH), :], sems.at[NXB + 1])
    wq_copy = pltpu.make_async_copy(wq_hbm, wq_scr, sems.at[NXB + 2])
    w1_copy = pltpu.make_async_copy(w1T_hbm.at[pl.ds(0, FL), :], w1T_scr, sems.at[NXB + 3])
    w2_copy = pltpu.make_async_copy(w2_hbm.at[pl.ds(0, FL), :], w2_scr, sems.at[NXB + 4])
    wo_copy = pltpu.make_async_copy(wo_hbm, wo_scr, sems.at[NXB + 5])
    w1r_copy = pltpu.make_async_copy(w1T_hbm.at[pl.ds(FL, FR), :], w1r_scr.at[pl.ds(0, FR), :],
                                     sems.at[NXB + 6])
    w2r_copy = pltpu.make_async_copy(w2_hbm.at[pl.ds(FL, FR), :], w2r_scr.at[pl.ds(0, FR), :],
                                     sems.at[NXB + 7])

    def o_copy(k):
        r0 = _off(k, OB)
        return pltpu.make_async_copy(out_scr.at[pl.ds(r0, OB), :], o_hbm.at[pl.ds(r0, OB), :],
                                     osems.at[k])

    x_copy(0).start()
    wq_copy.start()
    wk_copy.start()
    wv_copy.start()
    x_copy(1).start()
    w1r_copy.start()
    for c in range(2, NXB):
        x_copy(c).start()
    w1r_scr[pl.ds(FR, FRP - FR), :] = jnp.zeros((FRP - FR, D), bf16)
    w2r_scr[pl.ds(FR, FRP - FR), :] = jnp.zeros((FRP - FR, D), bf16)

    def ln_piece(r0, n):
        xn_scr[r0 // 2:(r0 + n) // 2, :] = _pk(_ln(x_scr[r0:r0 + n, :]).astype(bf16))

    def q_mm(m):
        t, gq = divmod(m, QG)
        xn = _upk(xn_scr[t * 64:(t + 1) * 64, :])
        w = _upk(wqT_scr[gq * 64:(gq + 1) * 64, :])
        acc_scr[(m % 4) * 128:(m % 4 + 1) * 128, 0:128] = lax.dot_general(
            w, xn, NT, preferred_element_type=f32)

    def q_quant(m, st):
        t, gq = divmod(m, QG)
        for k in range(HG):
            hh = gq * HG + k
            q = acc_scr[(m % 4) * 128 + k * DH:(m % 4) * 128 + (k + 1) * DH, 0:128]
            n2 = jnp.sum(q * q, axis=0, keepdims=True) + 1e-36
            st["qn2"] = n2 if st["qn2"] is None else jnp.maximum(st["qn2"], n2)
            rs = lax.rsqrt(n2)
            sq_scr[hh:hh + 1, t * 128:(t + 1) * 128] = n2 * rs
            hi8, hi, lo, lo2 = _limbs(q * (rs * FS))
            q8 = jnp.concatenate([hi8, hi8, hi8, hi8, hi, lo, lo2, jnp.zeros_like(hi)], axis=0)
            q8_scr[hh, :, t * 128:(t + 1) * 128] = q8.astype(i8)

    def kv_mm(t, st):
        xn = _upk(xn_scr[t * 64:(t + 1) * 64, :])
        r = lax.dot_general(wkvT_scr[...], xn, NT, preferred_element_type=f32)
        kT = r[0:DH, :]
        kT_scr[:, t * 128:(t + 1) * 128] = kT
        vT_scr[:, t * 128:(t + 1) * 128] = _pk(r[DH:2 * DH, :].astype(bf16))
        am = jnp.abs(r)
        st["amax"] = am if st["amax"] is None else jnp.maximum(st["amax"], am)
        k2 = jnp.sum(kT * kT, axis=0, keepdims=True)
        st["kn2"] = k2 if st["kn2"] is None else jnp.maximum(st["kn2"], k2)

    def k_stats(st):
        amax = st["amax"]
        kmax = jnp.max(jnp.max(amax[0:DH, :], axis=0, keepdims=True), axis=1, keepdims=True)
        st["vmax"] = jnp.max(jnp.max(amax[DH:2 * DH, :], axis=0, keepdims=True), axis=1, keepdims=True)
        st["kn2"] = jnp.max(st["kn2"], axis=1, keepdims=True)
        kmax = jnp.maximum(kmax, 1e-30)
        st["kscale"] = FS / kmax
        sq_scr[H:H + 8, 0:TQ] = jnp.broadcast_to(kmax * (256.0 * CSC / (FS * FS)), (8, TQ))

    def k_quant(c, st):
        hi8, hi, lo, lo2 = _limbs(kT_scr[:, c * 128:(c + 1) * 128] * st["kscale"])
        k8T = jnp.concatenate([hi8, hi8, hi8, hi8, lo, hi, lo2, jnp.zeros_like(hi)], axis=0)
        k8_scr[c * 128:(c + 1) * 128, :] = k8T.T.astype(i8)

    def repack(j):
        w1p_scr[:, j * 128:(j + 1) * 128] = _pk(w1T_scr[j * 128:(j + 1) * 128, :].T)
        w2p_scr[j * 64:(j + 1) * 64, :] = _pk(w2_scr[j * 128:(j + 1) * 128, :])

    def up_rest(u):
        t, j = divmod(u, FRP // 128)
        xk = _upk(xn_scr[t * 64:(t + 1) * 64, :])
        hh = lax.dot_general(xk, w1r_scr[j * 128:(j + 1) * 128, :], NT, preferred_element_type=f32)
        hr_scr[t * 64:(t + 1) * 64, j * 128:(j + 1) * 128] = _pk(_silu(hh).astype(bf16))

    st = dict(amax=None, kn2=None, qn2=None)
    x_copy(0).wait()
    for r0 in range(0, XB[1], 32):
        ln_piece(r0, 32)
    ln_done = XB[1]
    wq_copy.wait()
    wk_copy.wait()
    wv_copy.wait()
    slots = _prologue_slots()
    qslot = {i: m for m, (k, i) in enumerate(slots) if k == "q"}
    QLAG, WM = 3, 96
    guard_at = qslot[NM - 1] + QLAG + 1
    waited, kv_done, kq_done, rp_done, qq_done = 1, 0, 0, 0, 0
    kv_ready_at = {t: -10 for t in range(ln_done // 128)}
    stats_at = None
    ok = None
    for m, (kind, idx) in enumerate(slots):
        r1 = min(S, ln_done + 32) if m >= 3 else ln_done
        if r1 > XB[waited]:
            x_copy(waited).wait()
            waited += 1
            if waited == 3:
                w1r_copy.wait()
            if waited == NXB:
                w1_copy.start()
                w2_copy.start()
                wo_copy.start()
                w2r_copy.start()
        if m == WM:
            w1_copy.wait()
            w2_copy.wait()
        if m == 0:
            wqT_scr[0:64, :] = _pk(wq_scr[:, 0:128].T)
        if m + 1 < QG:
            wqT_scr[(m + 1) * 64:(m + 2) * 64, :] = _pk(wq_scr[:, (m + 1) * 128:(m + 2) * 128].T)
        if kind == "q":
            assert (idx // QG + 1) * 128 <= ln_done and idx - qq_done < 4
            q_mm(idx)
        else:
            assert waited >= 3 and (idx // (FRP // 128) + 1) * 128 <= ln_done
            up_rest(idx)
        if kv_done < NTL and kv_done in kv_ready_at and m >= kv_ready_at[kv_done] + 2:
            kv_mm(kv_done, st)
            kv_done += 1
            if kv_done == NTL:
                stats_at = m + 2
        if qq_done < NM and m >= qslot[qq_done] + QLAG:
            q_quant(qq_done, st)
            qq_done += 1
        if stats_at is not None and m == stats_at:
            k_stats(st)
        if stats_at is not None and m >= stats_at + 2 and kq_done < NTL:
            k_quant(kq_done, st)
            kq_done += 1
        if m >= WM and rp_done < JL and (m - WM) % 2 == 0:
            repack(rp_done)
            rp_done += 1
        if 80 <= m < 96:
            z = m - 80
            p_scr[1, z * 64:(z + 1) * 64, :] = jnp.zeros((64, TQ), u32)
            if z == 0:
                l_scr[1] = jnp.ones((8, TQ), f32)
        if m == guard_at:
            bound2 = jnp.max(st["qn2"], axis=1, keepdims=True) * st["kn2"] * (CSC * CSC)
            safe = ((bound2 <= BMAX * BMAX) & (st["vmax"] <= 2.0 ** 40) & (st["vmax"] >= 2.0 ** -30))
            ok = jnp.where(safe, 1, 0).astype(i32)[0, 0] > 0
        if r1 > ln_done:
            ln_piece(ln_done, 32)
            if r1 % 128 == 0:
                kv_ready_at[r1 // 128 - 1] = m
            ln_done = r1
    assert kq_done == NTL and rp_done == JL and qq_done == NM and ok is not None
    wo_copy.wait()
    w2r_copy.wait()

    def qk(h, g, c, slot, lacc, sq):
        q = q8_scr[h, :, g * TQ:(g + 1) * TQ]
        s = jnp.dot(k8_scr[c * KC:(c + 2) * KC, :], q, preferred_element_type=i32).astype(f32)
        p = jnp.exp2(s * sq)
        ls = jnp.sum(p.reshape(2 * KC // 8, 8, TQ), axis=0)
        P[slot][c * KC // 2:(c + 2) * KC // 2, :] = _pk(p.astype(bf16))
        return ls if lacc is None else lacc + ls

    def pv(c, slot, acc):
        p = _upk(P[slot][c * KC // 2:(c + 1) * KC // 2, :])
        v = _upk(vT_scr[:, c * KC:(c + 1) * KC])
        o = jnp.dot(v, p, preferred_element_type=f32)
        return o if acc is None else o + acc

    def ffn_piece(rs_idx, t, hslot):
        j = t // 2
        r0 = _off(rs_idx, RS)
        h0 = hslot * (RS // 2)
        if t % 2 == 0:
            xk = _upk(xn_scr[pl.ds(_off(rs_idx, RS // 2), RS // 2), :])
            hh = jnp.dot(xk, _upk(w1p_scr[:, j * 128:(j + 1) * 128]), preferred_element_type=f32)
            hid_scr[h0:h0 + RS // 2, j * 128:(j + 1) * 128] = _pk(_silu(hh).astype(bf16))
        else:
            hb = _upk(hid_scr[h0:h0 + RS // 2, j * 128:(j + 1) * 128])
            part = jnp.dot(hb, _upk(w2p_scr[j * 64:(j + 1) * 64, :]), preferred_element_type=f32)
            if j == 0:
                acc_scr[pl.ds(r0, RS), :] = part + x_scr[pl.ds(r0, RS), :].astype(f32)
            else:
                acc_scr[pl.ds(r0, RS), :] = acc_scr[pl.ds(r0, RS), :] + part

    def stage(hq, gq, q_slot, hp, gp, p_slot, filler):
        acc = None
        lacc = None
        if hq is not None:
            sq = sq_scr[pl.ds(hq, 1), gq * TQ:(gq + 1) * TQ] * sq_scr[H:H + 1, 0:TQ]
        for c in range(0, NC, 2):
            if hq is not None:
                lacc = qk(hq, gq, c, q_slot, lacc, sq)
            else:
                filler.pop(0)()
            acc = pv(c, p_slot, acc)
            filler.pop(0)()
            acc = pv(c + 1, p_slot, acc)
        if hq is not None:
            L[q_slot][...] = lacc
        l = jnp.sum(L[p_slot][...], axis=0, keepdims=True)
        oT_scr[pl.ds(_off(hp + 1, 8), 8), gp * TQ:(gp + 1) * TQ] = _pk((acc / l).astype(bf16))

    def fin_a(k):
        hb = _upk(hr_scr[pl.ds(_off(k, OB // 2), OB // 2), :])
        part = jnp.dot(hb, w2r_scr[...], preferred_element_type=f32)
        acc_scr[pl.ds(_off(k, OB), OB), :] = acc_scr[pl.ds(_off(k, OB), OB), :] + part

    def fin_b(k):
        oT = _upk(oT_scr[8:8 + D // 2, pl.ds(_off(k, OB), OB)])
        attn = lax.dot_general(oT, wo_scr[...], TN, preferred_element_type=f32)
        out_scr[pl.ds(_off(k, OB), OB), :] = (attn + acc_scr[pl.ds(_off(k, OB), OB), :]).astype(bf16)
        o_copy(k).start()

    @pl.when(ok)
    def _fast():
        nsub = RB // RS

        def body(it, carry):
            fl = [functools.partial(ffn_piece, it * nsub + sb, t, sb)
                  for t in _ffn_order() for sb in range(nsub)]
            for u in range(HB * NG):
                h, g = it * HB + u // NG, u % NG
                hp, gp = (h - 1, NG - 1) if g == 0 else (h, g - 1)
                stage(h, g, u % 2, hp, gp, (u + 1) % 2, fl)
            assert not fl
            return carry

        lax.fori_loop(0, H // HB, body, 0)
        stage(None, None, None, H - 1, NG - 1, 1, [functools.partial(fin_a, k) for k in range(NO)])
        for k in range(NO):
            fin_b(k)

    @pl.when(jnp.logical_not(ok))
    def _slow():
        def kbody(t, carry):
            xn = _upk(xn_scr[pl.ds(_off(t, 64), 64), :])
            kb_scr[pl.ds(_off(t, 128), 128), :] = lax.dot_general(
                xn, wkvT_scr[0:DH, :], NT, preferred_element_type=f32).astype(bf16)
            return carry

        lax.fori_loop(0, NTL, kbody, 0)

        def head(idx, carry):
            t = idx // H
            h = idx % H
            w = _upk(wqT_scr[pl.ds(_off(h, DH // 2), DH // 2), :])
            xn = _upk(xn_scr[pl.ds(_off(t, 64), 64), :])
            q = (lax.dot_general(w, xn, NT, preferred_element_type=f32) * CSC).astype(bf16)
            sT = jnp.dot(kb_scr[...], q, preferred_element_type=f32)
            p = jnp.exp2(sT - jnp.max(sT, axis=0, keepdims=True))
            l = jnp.sum(p, axis=0, keepdims=True)
            oT = jnp.dot(_upk(vT_scr[...]), p.astype(bf16), preferred_element_type=f32)
            oT_scr[pl.ds(_off(h + 1, 8), 8), pl.ds(_off(t, 128), 128)] = _pk((oT / l).astype(bf16))
            return carry

        lax.fori_loop(0, H * NTL, head, 0)

        def fbody(r, carry):
            for t in _ffn_order():
                ffn_piece(r, t, 0)
            return carry

        lax.fori_loop(0, S // RS, fbody, 0)

        def obody(k, carry):
            fin_a(k)
            fin_b(k)
            return carry

        lax.fori_loop(0, NO, obody, 0)

    for k in range(NO):
        o_copy(k).wait()


@jax.jit
def pallas_parallel_sum__grouped_kv_mqa__dense_activation_silu__prompt_kernel(
    A_x: jax.Array,
    A_wq: jax.Array,
    A_wk: jax.Array,
    A_wv: jax.Array,
    A_wo: jax.Array,
    B_x: jax.Array,
    B_w1: jax.Array,
    B_w2: jax.Array,
):
    del B_x
    anyspec = pl.BlockSpec(memory_space=pl.ANY)
    out = pl.pallas_call(
        _kernel,
        in_specs=[anyspec] * 7,
        out_specs=anyspec,
        out_shape=jax.ShapeDtypeStruct((S, D), bf16),
        scratch_shapes=[
            pltpu.VMEM((S, D), bf16),
            pltpu.VMEM((D, D), bf16),
            pltpu.VMEM((2 * DH, D), bf16),
            pltpu.VMEM((D, D), bf16),
            pltpu.VMEM((FL, D), bf16),
            pltpu.VMEM((FL, D), bf16),
            pltpu.VMEM((FRP, D), bf16),
            pltpu.VMEM((FRP, D), bf16),
            pltpu.SemaphoreType.DMA((NXB + 8,)),
            pltpu.SemaphoreType.DMA((NO,)),
            pltpu.VMEM((S // 2, D), u32),
            pltpu.VMEM((D // 2, D), u32),
            pltpu.VMEM((DH, S), f32),
            pltpu.VMEM((S, 128), i8),
            pltpu.VMEM((S, DH), bf16),
            pltpu.VMEM((DH // 2, S), u32),
            pltpu.VMEM((H, 128, S), i8),
            pltpu.VMEM((H + 8, S), f32),
            pltpu.VMEM(((H + 1) * 8, S), u32),
            pltpu.VMEM((S, D), f32),
            pltpu.VMEM((RB // 2, FL), u32),
            pltpu.VMEM((S // 2, FRP), u32),
            pltpu.VMEM((2, S // 2, TQ), u32),
            pltpu.VMEM((2, 8, TQ), f32),
            pltpu.VMEM((S, D), bf16),
            pltpu.VMEM((D // 2, FL), u32),
            pltpu.VMEM((FL // 2, D), u32),
        ],
        compiler_params=pltpu.CompilerParams(vmem_limit_bytes=100 * 1024 * 1024),
    )(A_x.reshape(S, D), A_wq, A_wk.T, A_wv.T, A_wo, B_w1.T, B_w2)
    return out.reshape(1, S, D)
```

```python
import functools
import math

import jax
import jax.numpy as jnp
from jax import lax
from jax.experimental import pallas as pl
from jax.experimental.pallas import tpu as pltpu

S, D, H, DH, F = 2048, 512, 32, 16, 1376
LOG2E = math.log2(math.e)
CSC = DH ** -0.5 * LOG2E
FS = 3960.0
BMAX = 64.0
MAGIC = 12582912.0
f32, bf16, i32, i8, u32 = jnp.float32, jnp.bfloat16, jnp.int32, jnp.int8, jnp.uint32
NT = (((1,), (1,)), ((), ()))
TN = (((0,), (0,)), ((), ()))

TQ, KC = 512, 256
NG, NC = S // TQ, S // KC
HB = 4
RB = S // (H // HB)
RS = 64
JL = 8
FL = JL * 128
FR, FRP = F - FL, 384
XB = (0, 256, 512, 1024, 2048)
NXB = len(XB) - 1
OB = 256
NO = S // OB
QG = 4
HG = H // QG
NTL = S // 128
NM = NTL * QG
NU = NTL * (FRP // 128)


def _ln(x):
    x = x.astype(f32)
    m = jnp.mean(x, axis=-1, keepdims=True)
    xc = x - m
    v = jnp.mean(xc * xc, axis=-1, keepdims=True)
    return xc * lax.rsqrt(v + 1e-5)


def _limbs(y):
    bits = pltpu.bitcast(y + MAGIC, i32)
    hi = (bits + 128) >> 8
    lo2 = (((bits << 24) >> 24) + 8) >> 4
    return hi << 3, hi, bits, lo2


def _silu(h):
    d = 1.0 + jnp.exp2(jnp.minimum(h * (-LOG2E), 126.0))
    r = pl.reciprocal(d, approx=True)
    r = r * (2.0 - d * r)
    return h * r


def _pk(x):
    return pltpu.bitcast(x, u32)


def _upk(x):
    return pltpu.bitcast(x, bf16)


def _off(k, n):
    return k * n if isinstance(k, int) else pl.multiple_of(k * n, n)


def _prologue_slots():
    slots, nq, nu = [], 0, 0
    while nq < NM or nu < NU:
        if nq < NM and (len(slots) < 12 or nu >= NU - 6 or nu * 4 >= (nq - 12) * 3):
            slots.append(("q", nq))
            nq += 1
        else:
            slots.append(("u", nu))
            nu += 1
    return slots


def _ffn_order():
    order = [0, 2]
    for j in range(JL):
        order.append(2 * j + 1)
        if j + 2 < JL:
            order.append(2 * (j + 2))
    return order


def _kernel(x_hbm, wq_hbm, wkT_hbm, wvT_hbm, wo_hbm, w1T_hbm, w2_hbm, o_hbm,
            x_scr, wq_scr, wkvT_scr, wo_scr, w1T_scr, w2_scr, w1r_scr, w2r_scr, sems, osems,
            xn_scr, wqT_scr, kT_scr, k8_scr, kb_scr, vT_scr,
            q8_scr, sq_scr, oT_scr, acc_scr, hid_scr, hr_scr, p_scr, l_scr, out_scr,
            w1p_scr, w2p_scr):
    P = [p_scr.at[k] for k in range(2)]
    L = [l_scr.at[k] for k in range(2)]

    def x_copy(c):
        lo, n = XB[c], XB[c + 1] - XB[c]
        return pltpu.make_async_copy(x_hbm.at[pl.ds(lo, n), :], x_scr.at[pl.ds(lo, n), :], sems.at[c])

    wk_copy = pltpu.make_async_copy(wkT_hbm, wkvT_scr.at[pl.ds(0, DH), :], sems.at[NXB])
    wv_copy = pltpu.make_async_copy(wvT_hbm, wkvT_scr.at[pl.ds(DH, DH), :], sems.at[NXB + 1])
    wq_copy = pltpu.make_async_copy(wq_hbm, wq_scr, sems.at[NXB + 2])
    w1_copy = pltpu.make_async_copy(w1T_hbm.at[pl.ds(0, FL), :], w1T_scr, sems.at[NXB + 3])
    w2_copy = pltpu.make_async_copy(w2_hbm.at[pl.ds(0, FL), :], w2_scr, sems.at[NXB + 4])
    wo_copy = pltpu.make_async_copy(wo_hbm, wo_scr, sems.at[NXB + 5])
    w1r_copy = pltpu.make_async_copy(w1T_hbm.at[pl.ds(FL, FR), :], w1r_scr.at[pl.ds(0, FR), :],
                                     sems.at[NXB + 6])
    w2r_copy = pltpu.make_async_copy(w2_hbm.at[pl.ds(FL, FR), :], w2r_scr.at[pl.ds(0, FR), :],
                                     sems.at[NXB + 7])

    def o_copy(k):
        r0 = _off(k, OB)
        return pltpu.make_async_copy(out_scr.at[pl.ds(r0, OB), :], o_hbm.at[pl.ds(r0, OB), :],
                                     osems.at[k])

    x_copy(0).start()
    wq_copy.start()
    wk_copy.start()
    wv_copy.start()
    x_copy(1).start()
    w1r_copy.start()
    for c in range(2, NXB):
        x_copy(c).start()
    w1r_scr[pl.ds(FR, FRP - FR), :] = jnp.zeros((FRP - FR, D), bf16)
    w2r_scr[pl.ds(FR, FRP - FR), :] = jnp.zeros((FRP - FR, D), bf16)
    p_scr[1] = jnp.zeros((S // 2, TQ), u32)
    l_scr[1] = jnp.ones((8, TQ), f32)

    def ln_piece(r0, n):
        xn_scr[r0 // 2:(r0 + n) // 2, :] = _pk(_ln(x_scr[r0:r0 + n, :]).astype(bf16))

    def q_mm(m):
        t, gq = divmod(m, QG)
        xn = _upk(xn_scr[t * 64:(t + 1) * 64, :])
        w = _upk(wqT_scr[gq * 64:(gq + 1) * 64, :])
        acc_scr[(m % 4) * 128:(m % 4 + 1) * 128, 0:128] = lax.dot_general(
            w, xn, NT, preferred_element_type=f32)

    def q_quant(m, st):
        t, gq = divmod(m, QG)
        for k in range(HG):
            hh = gq * HG + k
            q = acc_scr[(m % 4) * 128 + k * DH:(m % 4) * 128 + (k + 1) * DH, 0:128]
            n2 = jnp.sum(q * q, axis=0, keepdims=True) + 1e-36
            st["qn2"] = n2 if st["qn2"] is None else jnp.maximum(st["qn2"], n2)
            rs = lax.rsqrt(n2)
            sq_scr[hh:hh + 1, t * 128:(t + 1) * 128] = n2 * rs
            hi8, hi, lo, lo2 = _limbs(q * (rs * FS))
            q8 = jnp.concatenate([hi8, hi8, hi8, hi8, hi, lo, lo2, jnp.zeros_like(hi)], axis=0)
            q8_scr[hh, :, t * 128:(t + 1) * 128] = q8.astype(i8)

    def kv_mm(t, st):
        xn = _upk(xn_scr[t * 64:(t + 1) * 64, :])
        r = lax.dot_general(wkvT_scr[...], xn, NT, preferred_element_type=f32)
        kT = r[0:DH, :]
        kT_scr[:, t * 128:(t + 1) * 128] = kT
        vT_scr[:, t * 128:(t + 1) * 128] = _pk(r[DH:2 * DH, :].astype(bf16))
        am = jnp.abs(r)
        st["amax"] = am if st["amax"] is None else jnp.maximum(st["amax"], am)
        k2 = jnp.sum(kT * kT, axis=0, keepdims=True)
        st["kn2"] = k2 if st["kn2"] is None else jnp.maximum(st["kn2"], k2)

    def k_stats(st):
        amax = st["amax"]
        kmax = jnp.max(jnp.max(amax[0:DH, :], axis=0, keepdims=True), axis=1, keepdims=True)
        st["vmax"] = jnp.max(jnp.max(amax[DH:2 * DH, :], axis=0, keepdims=True), axis=1, keepdims=True)
        st["kn2"] = jnp.max(st["kn2"], axis=1, keepdims=True)
        kmax = jnp.maximum(kmax, 1e-30)
        st["kscale"] = FS / kmax
        sq_scr[H:H + 8, 0:TQ] = jnp.broadcast_to(kmax * (256.0 * CSC / (FS * FS)), (8, TQ))

    def k_quant(c, st):
        hi8, hi, lo, lo2 = _limbs(kT_scr[:, c * 128:(c + 1) * 128] * st["kscale"])
        k8T = jnp.concatenate([hi8, hi8, hi8, hi8, lo, hi, lo2, jnp.zeros_like(hi)], axis=0)
        k8_scr[c * 128:(c + 1) * 128, :] = k8T.T.astype(i8)

    def repack(j):
        w1p_scr[:, j * 128:(j + 1) * 128] = _pk(w1T_scr[j * 128:(j + 1) * 128, :].T)
        w2p_scr[j * 64:(j + 1) * 64, :] = _pk(w2_scr[j * 128:(j + 1) * 128, :])

    def up_rest(u):
        t, j = divmod(u, FRP // 128)
        xk = _upk(xn_scr[t * 64:(t + 1) * 64, :])
        hh = lax.dot_general(xk, w1r_scr[j * 128:(j + 1) * 128, :], NT, preferred_element_type=f32)
        hr_scr[t * 64:(t + 1) * 64, j * 128:(j + 1) * 128] = _pk(_silu(hh).astype(bf16))

    st = dict(amax=None, kn2=None, qn2=None)
    x_copy(0).wait()
    for r0 in range(0, XB[1], 32):
        ln_piece(r0, 32)
    ln_done = XB[1]
    wq_copy.wait()
    wk_copy.wait()
    wv_copy.wait()
    slots = _prologue_slots()
    qslot = {i: m for m, (k, i) in enumerate(slots) if k == "q"}
    QLAG, WM = 3, 96
    guard_at = qslot[NM - 1] + QLAG + 1
    waited, kv_done, kq_done, rp_done, qq_done = 1, 0, 0, 0, 0
    kv_ready_at = {t: -10 for t in range(ln_done // 128)}
    stats_at = None
    ok = None
    for m, (kind, idx) in enumerate(slots):
        r1 = min(S, ln_done + 32) if m >= 3 else ln_done
        if r1 > XB[waited]:
            x_copy(waited).wait()
            waited += 1
            if waited == 3:
                w1r_copy.wait()
            if waited == NXB:
                w1_copy.start()
                w2_copy.start()
                wo_copy.start()
                w2r_copy.start()
        if m == WM:
            w1_copy.wait()
            w2_copy.wait()
        if m == 0:
            wqT_scr[0:64, :] = _pk(wq_scr[:, 0:128].T)
        if m + 1 < QG:
            wqT_scr[(m + 1) * 64:(m + 2) * 64, :] = _pk(wq_scr[:, (m + 1) * 128:(m + 2) * 128].T)
        if kind == "q":
            assert (idx // QG + 1) * 128 <= ln_done and idx - qq_done < 4
            q_mm(idx)
        else:
            assert waited >= 3 and (idx // (FRP // 128) + 1) * 128 <= ln_done
            up_rest(idx)
        if kv_done < NTL and kv_done in kv_ready_at and m >= kv_ready_at[kv_done] + 2:
            kv_mm(kv_done, st)
            kv_done += 1
            if kv_done == NTL:
                stats_at = m + 2
        if qq_done < NM and m >= qslot[qq_done] + QLAG:
            q_quant(qq_done, st)
            qq_done += 1
        if stats_at is not None and m == stats_at:
            k_stats(st)
        if stats_at is not None and m >= stats_at + 2 and kq_done < NTL:
            k_quant(kq_done, st)
            kq_done += 1
        if m >= WM and rp_done < JL and (m - WM) % 2 == 0:
            repack(rp_done)
            rp_done += 1
        if m == guard_at:
            bound2 = jnp.max(st["qn2"], axis=1, keepdims=True) * st["kn2"] * (CSC * CSC)
            safe = ((bound2 <= BMAX * BMAX) & (st["vmax"] <= 2.0 ** 40) & (st["vmax"] >= 2.0 ** -30))
            ok = jnp.where(safe, 1, 0).astype(i32)[0, 0] > 0
        if r1 > ln_done:
            ln_piece(ln_done, 32)
            if r1 % 128 == 0:
                kv_ready_at[r1 // 128 - 1] = m
            ln_done = r1
    assert kq_done == NTL and rp_done == JL and qq_done == NM and ok is not None
    wo_copy.wait()
    w2r_copy.wait()

    def qk(h, g, c, slot, lacc, sq):
        q = q8_scr[h, :, g * TQ:(g + 1) * TQ]
        s = jnp.dot(k8_scr[c * KC:(c + 2) * KC, :], q, preferred_element_type=i32).astype(f32)
        p = jnp.exp2(s * sq)
        ls = jnp.sum(p.reshape(2 * KC // 8, 8, TQ), axis=0)
        P[slot][c * KC // 2:(c + 2) * KC // 2, :] = _pk(p.astype(bf16))
        return ls if lacc is None else lacc + ls

    def pv(c, slot, acc):
        p = _upk(P[slot][c * KC // 2:(c + 1) * KC // 2, :])
        v = _upk(vT_scr[:, c * KC:(c + 1) * KC])
        o = jnp.dot(v, p, preferred_element_type=f32)
        return o if acc is None else o + acc

    def ffn_piece(rs_idx, t, hslot):
        j = t // 2
        r0 = _off(rs_idx, RS)
        h0 = hslot * (RS // 2)
        if t % 2 == 0:
            xk = _upk(xn_scr[pl.ds(_off(rs_idx, RS // 2), RS // 2), :])
            hh = jnp.dot(xk, _upk(w1p_scr[:, j * 128:(j + 1) * 128]), preferred_element_type=f32)
            hid_scr[h0:h0 + RS // 2, j * 128:(j + 1) * 128] = _pk(_silu(hh).astype(bf16))
        else:
            hb = _upk(hid_scr[h0:h0 + RS // 2, j * 128:(j + 1) * 128])
            part = jnp.dot(hb, _upk(w2p_scr[j * 64:(j + 1) * 64, :]), preferred_element_type=f32)
            if j == 0:
                acc_scr[pl.ds(r0, RS), :] = part + x_scr[pl.ds(r0, RS), :].astype(f32)
            else:
                acc_scr[pl.ds(r0, RS), :] = acc_scr[pl.ds(r0, RS), :] + part

    def stage(hq, gq, q_slot, hp, gp, p_slot, filler):
        acc = None
        lacc = None
        if hq is not None:
            sq = sq_scr[pl.ds(hq, 1), gq * TQ:(gq + 1) * TQ] * sq_scr[H:H + 1, 0:TQ]
        for c in range(0, NC, 2):
            if hq is not None:
                lacc = qk(hq, gq, c, q_slot, lacc, sq)
            else:
                filler.pop(0)()
            acc = pv(c, p_slot, acc)
            filler.pop(0)()
            acc = pv(c + 1, p_slot, acc)
        if hq is not None:
            L[q_slot][...] = lacc
        l = jnp.sum(L[p_slot][...], axis=0, keepdims=True)
        oT_scr[pl.ds(_off(hp + 1, 8), 8), gp * TQ:(gp + 1) * TQ] = _pk((acc / l).astype(bf16))

    def fin_a(k):
        hb = _upk(hr_scr[pl.ds(_off(k, OB // 2), OB // 2), :])
        part = jnp.dot(hb, w2r_scr[...], preferred_element_type=f32)
        acc_scr[pl.ds(_off(k, OB), OB), :] = acc_scr[pl.ds(_off(k, OB), OB), :] + part

    def fin_b(k):
        oT = _upk(oT_scr[8:8 + D // 2, pl.ds(_off(k, OB), OB)])
        attn = lax.dot_general(oT, wo_scr[...], TN, preferred_element_type=f32)
        out_scr[pl.ds(_off(k, OB), OB), :] = (attn + acc_scr[pl.ds(_off(k, OB), OB), :]).astype(bf16)
        o_copy(k).start()

    @pl.when(ok)
    def _fast():
        nsub = RB // RS

        def body(it, carry):
            fl = [functools.partial(ffn_piece, it * nsub + sb, t, sb)
                  for t in _ffn_order() for sb in range(nsub)]
            for u in range(HB * NG):
                h, g = it * HB + u // NG, u % NG
                hp, gp = (h - 1, NG - 1) if g == 0 else (h, g - 1)
                stage(h, g, u % 2, hp, gp, (u + 1) % 2, fl)
            assert not fl
            return carry

        lax.fori_loop(0, H // HB, body, 0)
        stage(None, None, None, H - 1, NG - 1, 1, [functools.partial(fin_a, k) for k in range(NO)])
        for k in range(NO):
            fin_b(k)

    @pl.when(jnp.logical_not(ok))
    def _slow():
        def kbody(t, carry):
            xn = _upk(xn_scr[pl.ds(_off(t, 64), 64), :])
            kb_scr[pl.ds(_off(t, 128), 128), :] = lax.dot_general(
                xn, wkvT_scr[0:DH, :], NT, preferred_element_type=f32).astype(bf16)
            return carry

        lax.fori_loop(0, NTL, kbody, 0)

        def head(idx, carry):
            t = idx // H
            h = idx % H
            w = _upk(wqT_scr[pl.ds(_off(h, DH // 2), DH // 2), :])
            xn = _upk(xn_scr[pl.ds(_off(t, 64), 64), :])
            q = (lax.dot_general(w, xn, NT, preferred_element_type=f32) * CSC).astype(bf16)
            sT = jnp.dot(kb_scr[...], q, preferred_element_type=f32)
            p = jnp.exp2(sT - jnp.max(sT, axis=0, keepdims=True))
            l = jnp.sum(p, axis=0, keepdims=True)
            oT = jnp.dot(_upk(vT_scr[...]), p.astype(bf16), preferred_element_type=f32)
            oT_scr[pl.ds(_off(h + 1, 8), 8), pl.ds(_off(t, 128), 128)] = _pk((oT / l).astype(bf16))
            return carry

        lax.fori_loop(0, H * NTL, head, 0)

        def fbody(r, carry):
            for t in _ffn_order():
                ffn_piece(r, t, 0)
            return carry

        lax.fori_loop(0, S // RS, fbody, 0)

        def obody(k, carry):
            fin_a(k)
            fin_b(k)
            return carry

        lax.fori_loop(0, NO, obody, 0)

    for k in range(NO):
        o_copy(k).wait()


@jax.jit
def pallas_parallel_sum__grouped_kv_mqa__dense_activation_silu__prompt_kernel(
    A_x: jax.Array,
    A_wq: jax.Array,
    A_wk: jax.Array,
    A_wv: jax.Array,
    A_wo: jax.Array,
    B_x: jax.Array,
    B_w1: jax.Array,
    B_w2: jax.Array,
):
    del B_x
    anyspec = pl.BlockSpec(memory_space=pl.ANY)
    out = pl.pallas_call(
        _kernel,
        in_specs=[anyspec] * 7,
        out_specs=anyspec,
        out_shape=jax.ShapeDtypeStruct((S, D), bf16),
        scratch_shapes=[
            pltpu.VMEM((S, D), bf16),
            pltpu.VMEM((D, D), bf16),
            pltpu.VMEM((2 * DH, D), bf16),
            pltpu.VMEM((D, D), bf16),
            pltpu.VMEM((FL, D), bf16),
            pltpu.VMEM((FL, D), bf16),
            pltpu.VMEM((FRP, D), bf16),
            pltpu.VMEM((FRP, D), bf16),
            pltpu.SemaphoreType.DMA((NXB + 8,)),
            pltpu.SemaphoreType.DMA((NO,)),
            pltpu.VMEM((S // 2, D), u32),
            pltpu.VMEM((D // 2, D), u32),
            pltpu.VMEM((DH, S), f32),
            pltpu.VMEM((S, 128), i8),
            pltpu.VMEM((S, DH), bf16),
            pltpu.VMEM((DH // 2, S), u32),
            pltpu.VMEM((H, 128, S), i8),
            pltpu.VMEM((H + 8, S), f32),
            pltpu.VMEM(((H + 1) * 8, S), u32),
            pltpu.VMEM((S, D), f32),
            pltpu.VMEM((RB // 2, FL), u32),
            pltpu.VMEM((S // 2, FRP), u32),
            pltpu.VMEM((2, S // 2, TQ), u32),
            pltpu.VMEM((2, 8, TQ), f32),
            pltpu.VMEM((S, D), bf16),
            pltpu.VMEM((D // 2, FL), u32),
            pltpu.VMEM((FL // 2, D), u32),
        ],
        compiler_params=pltpu.CompilerParams(vmem_limit_bytes=100 * 1024 * 1024),
    )(A_x.reshape(S, D), A_wq, A_wk.T, A_wv.T, A_wo, B_w1.T, B_w2)
    return out.reshape(1, S, D)
```
